```python
import os as _os
_os.environ.setdefault("JAX_PLATFORMS", "cpu")
import jax
import jax.numpy as jnp

def _softmax(x, axis=-1):
    return jax.nn.softmax(x, axis=axis)
def _gelu(x):
    return jax.nn.gelu(x, approximate=True)
def _silu(x):
    return jax.nn.silu(x)
def _sigmoid(x):
    return jax.nn.sigmoid(x)
def _layernorm(x, axis=-1, eps=1e-5):
    m = jnp.mean(x, axis=axis, keepdims=True)
    v = jnp.var(x, axis=axis, keepdims=True)
    return (x - m) / jnp.sqrt(v + eps)
def _scatter_add(tgt, idx, src, axis=0):
    return tgt.at[idx].add(src)
def _segment_sum(src, seg, n):
    return jax.ops.segment_sum(src, seg, n)
class _Rng:
    def __init__(self, key):
        self._k = key
    def _next(self):
        self._k, sub = jax.random.split(self._k)
        return sub
    def normal(self, shape):
        return jax.random.normal(self._next(), shape, dtype=jnp.bfloat16)
    def randint(self, lo, hi, shape):
        return jax.random.randint(self._next(), shape, lo, hi, dtype=jnp.int32)
    def uniform(self, shape, lo=0.0, hi=1.0):
        return jax.random.uniform(self._next(), shape, jnp.bfloat16, lo, hi)
    def permutation(self, n):
        return jax.random.permutation(self._next(), n)


kernel_name = 'sequential_preLN__softmax_full_mha__mixer_channel_mlp__prompt'

def setup_inputs():
    _rng = _Rng(jax.random.key(int.from_bytes(__import__("os").urandom(4), "little")))
    _w = (lambda a: (lambda t: t.astype(jnp.bfloat16) if jnp.issubdtype(t.dtype, jnp.floating) else t)(jnp.asarray(a)))
    def _A_setup():
        B, S, D = 1, 2048, 1024
        return {
            "x": _w((lambda *s: _rng.normal(s) * 0.05)(B, S, D)),
            "wqkv": _w((lambda *s: _rng.normal(s) * 0.05)(D, 3 * D)),
            "wo": _w((lambda *s: _rng.normal(s) * 0.05)(D, D)),
        }
    _A_in = _A_setup()

    def _B_setup():
        B, S, D, F = 1, 2048, 1024, 3584
        return {
            "x": _w((lambda *s: _rng.normal(s) * 0.05)(B, S, D)),
            "w1": _w((lambda *s: _rng.normal(s) * 0.8)(D, F) * (D ** -0.5)),
            "b1": _w((lambda *s: _rng.normal(s) * 0.8)(F)),
            "w2": _w((lambda *s: _rng.normal(s) * 0.8)(F, D) * (F ** -0.5)),
            "b2": _w((lambda *s: _rng.normal(s) * 0.05)(D)),
        }
    _B_in = _B_setup()

    return {
        "A_x": _A_in["x"],
        "A_wqkv": _A_in["wqkv"],
        "A_wo": _A_in["wo"],
        "B_x": _B_in["x"],
        "B_w1": _B_in["w1"],
        "B_b1": _B_in["b1"],
        "B_w2": _B_in["w2"],
        "B_b2": _B_in["b2"],
    }

def reference(A_x, A_wqkv, A_wo, B_x, B_w1, B_b1, B_w2, B_b2):
    def _A_ref(x, wqkv, wo):
        B, S, D = x.shape
        H = 32; Dh = D // H
        qkv = (lambda x, *d: x.transpose(*d))((x @ wqkv).reshape(B, S, 3, H, Dh), 2, 0, 3, 1, 4)
        q, k, v = qkv[0], qkv[1], qkv[2]
        scale = Dh ** -0.5
        scores = jnp.einsum("bhqd,bhkd->bhqk", q, k) * scale
        p = _softmax(scores, axis=-1)
        o = jnp.einsum("bhqk,bhkd->bhqd", p, v)
        return (lambda x, *d: x.transpose(*d))(o, 0, 2, 1, 3).reshape(B, S, D) @ wo

    def _B_ref(x, w1, b1, w2, b2):
        y = _layernorm(x, axis=-1)
        h = _gelu(jnp.einsum("bsd,df->bsf", y, w1) + b1)
        return jnp.einsum("bsf,fd->bsd", h, w2) + b2

    x = A_x
    h = x + _A_ref(_layernorm(x, axis=-1), A_wqkv, A_wo)
    h2 = h + _B_ref(_layernorm(h, axis=-1), B_w1, B_b1, B_w2, B_b2)
    return h2
```

```python
import functools
import math

import jax
import jax.numpy as jnp
from jax import lax
import jax.experimental.pallas as pl
import jax.experimental.pallas.tpu as pltpu

S, D, H, DH, F = 2048, 1024, 32, 32, 3584
BQ = 512
NU = S // BQ
CK = 128
NC = S // CK
NT = BQ // 128
RB1 = 256
RB3 = 128
EPS = 1e-5
QSCALE = (DH ** -0.5) * math.log2(math.e)

bf16, f32, u32 = jnp.bfloat16, jnp.float32, jnp.uint32


def _pk(x):
    return pltpu.bitcast(x, u32)


def _upk(x):
    return pltpu.bitcast(x, bf16)


def _layernorm(x):
    m = jnp.mean(x, axis=-1, keepdims=True)
    xc = x - m
    v = jnp.mean(xc * xc, axis=-1, keepdims=True)
    return xc * lax.rsqrt(v + EPS)


def _gelu(x):
    c = math.sqrt(2.0 / math.pi)
    inner = x * (c + (c * 0.044715) * (x * x))
    hx = 0.5 * x
    return hx + hx * jnp.tanh(inner)


def _dot(a, b):
    return jnp.dot(a, b, preferred_element_type=f32)


def _kernel(x_hbm, wqkv_hbm, wo_hbm, w1_hbm, b1_ref, w2_hbm, b2_ref, o_hbm,
            x_s, wqkv_s, wo_s, w1_s, w2_s, xn_s, k_s, qt_s, vt_s, ot_s, out_s,
            qm0, qm1, qm2, qm3, sb0, sb1, sb2, sb3, ms_s, sem_x, sem_w, sem_o):
    qms = (qm0, qm1, qm2, qm3)
    sbs = (sb0, sb1, sb2, sb3)
    n1 = S // RB1

    def x_copy(r):
        return pltpu.make_async_copy(x_hbm.at[pl.ds(r * RB1, RB1)], x_s.at[pl.ds(r * RB1, RB1)], sem_x.at[r])

    def wqkv_copy(j):
        return pltpu.make_async_copy(wqkv_hbm.at[:, pl.ds(j * D, D)], wqkv_s.at[j], sem_w.at[j])

    wo_copy = pltpu.make_async_copy(wo_hbm, wo_s, sem_w.at[3])
    w1_copy = pltpu.make_async_copy(w1_hbm, w1_s, sem_w.at[4])
    w2_copy = pltpu.make_async_copy(w2_hbm, w2_s, sem_w.at[5])

    x_copy(0).start()
    wqkv_copy(1).start()
    x_copy(0).wait()
    for r in range(1, n1):
        x_copy(r).start()
    wqkv_copy(1).wait()
    wqkv_copy(0).start()
    wqkv_copy(2).start()

    def p1a(r, carry):
        @pl.when(r > 0)
        def _():
            x_copy(r).wait()
        sub = 128
        for a in range(RB1 // sub):
            row = pl.multiple_of(r * RB1 + a * sub, sub)
            xn = _layernorm(x_s[pl.ds(row, sub), :].astype(f32)).astype(bf16)
            xn_s[pl.ds(row, sub), :] = xn
            kk = _dot(xn, wqkv_s[1]).astype(bf16)
            prow = pl.multiple_of(r * (RB1 // 2) + a * (sub // 2), sub // 2)
            for g in range(D // 128):
                k_s[g, pl.ds(prow, sub // 2), :] = _pk(kk[:, g * 128:(g + 1) * 128])
        return carry

    lax.fori_loop(0, n1, p1a, 0)

    wqkv_copy(0).wait()
    wqkv_copy(2).wait()
    wo_copy.start()
    w1_copy.start()
    w2_copy.start()

    def p1b(r, carry):
        row = pl.multiple_of(r * RB1, RB1)
        xn = xn_s[pl.ds(row, RB1), :]
        q = _dot(xn, wqkv_s[0]) * QSCALE
        for t in range(RB1 // 128):
            qt_s[r * (RB1 // 128) + t] = _pk(q[t * 128:(t + 1) * 128, :].T.astype(bf16))
        v = _dot(xn, wqkv_s[2])
        for t in range(RB1 // 128):
            vt_s[r * (RB1 // 128) + t] = _pk(v[t * 128:(t + 1) * 128, :].T.astype(bf16))
        return carry

    lax.fori_loop(0, n1, p1b, 0)

    def prep_q(h, u):
        g = h // 4
        row = lax.broadcasted_iota(jnp.int32, (64, 128), 0) // (DH // 2)
        keep = row == (h % 4)
        for t in range(NT):
            q = qt_s[u * NT + t, pl.ds(pl.multiple_of(g * 64, 64), 64), :]
            qms[u][t] = jnp.where(keep, q, jnp.zeros_like(q))

    def qk_chunk(h, u, c, m8):
        kk = _upk(k_s[h // 4, c * (CK // 2):(c + 1) * (CK // 2), :])
        qm = jnp.concatenate([_upk(qms[u][t]) for t in range(NT)], axis=1)
        s = _dot(kk, qm)
        sbs[u][c * CK:(c + 1) * CK, :] = s
        for r in range(CK // 8):
            sr = s[r * 8:(r + 1) * 8]
            m8 = sr if m8 is None else jnp.maximum(m8, sr)
        return m8

    def pv_chunk(h, c, s, m, l8, acc):
        p = jnp.exp2(s - m)
        for r in reversed(range(CK // 8)):
            pr = p[r * 8:(r + 1) * 8]
            l8 = pr if l8 is None else l8 + pr
        vt = _upk(vt_s[c, pl.ds(pl.multiple_of(h * (DH // 2), DH // 2), DH // 2), :])
        o = _dot(vt, p.astype(bf16))
        return l8, (o if acc is None else acc + o)

    def finish(h, u, l8, acc):
        l = jnp.sum(l8, axis=0, keepdims=True)
        res = _pk((acc * (1.0 / l)).astype(bf16))
        for t in range(NT):
            ot_s[u * NT + t, pl.ds(pl.multiple_of(h * (DH // 2), DH // 2), DH // 2), :] = res[:, t * 128:(t + 1) * 128]

    for u in range(NU):
        prep_q(0, u)
        m8 = None
        for c in range(NC):
            m8 = qk_chunk(0, u, c, m8)
        ms_s[u] = jnp.max(m8, axis=0, keepdims=True)
        prep_q(1, u)

    def attn(h, carry):
        for u in range(NU):
            m = ms_s[u]
            m8 = l8 = acc = None
            for c in range(NC):
                s_old = sbs[u][c * CK:(c + 1) * CK, :]
                m8 = qk_chunk(h + 1, u, c, m8)
                l8, acc = pv_chunk(h, c, s_old, m, l8, acc)
            ms_s[u] = jnp.max(m8, axis=0, keepdims=True)
            prep_q(jnp.minimum(h + 2, H - 1), u)
            finish(h, u, l8, acc)
        return carry

    lax.fori_loop(0, H - 1, attn, 0)

    for u in range(NU):
        m = ms_s[u]
        l8 = acc = None
        for c in range(NC):
            l8, acc = pv_chunk(H - 1, c, sbs[u][c * CK:(c + 1) * CK, :], m, l8, acc)
        finish(H - 1, u, l8, acc)

    wo_copy.wait()
    w1_copy.wait()
    w2_copy.wait()

    def out_copy(r):
        return pltpu.make_async_copy(out_s.at[pl.ds(r * RB3, RB3)], o_hbm.at[pl.ds(r * RB3, RB3)], sem_o.at[r])

    def p3(r, carry):
        row = pl.multiple_of(r * RB3, RB3)
        o = _upk(ot_s[r]).T
        hres = x_s[pl.ds(row, RB3), :].astype(f32) + _dot(o, wo_s[...])
        y = _layernorm(hres).astype(bf16)
        b1 = b1_ref[...].astype(f32).reshape(1, F)
        b2 = b2_ref[...].astype(f32).reshape(1, D)
        g = _gelu(_dot(y, w1_s[...]) + b1).astype(bf16)
        res = hres + b2 + _dot(g, w2_s[...])
        out_s[pl.ds(row, RB3), :] = res.astype(bf16)
        out_copy(r).start()
        return carry

    lax.fori_loop(0, S // RB3, p3, 0)
    for r in range(S // RB3):
        out_copy(r).wait()


@jax.jit
def pallas_sequential_preLN__softmax_full_mha__mixer_channel_mlp__prompt_kernel(
    A_x: jax.Array,
    A_wqkv: jax.Array,
    A_wo: jax.Array,
    B_x: jax.Array,
    B_w1: jax.Array,
    B_b1: jax.Array,
    B_w2: jax.Array,
    B_b2: jax.Array,
):
    del B_x
    any_spec = pl.BlockSpec(memory_space=pl.ANY)
    vmem_spec = pl.BlockSpec(memory_space=pltpu.VMEM)
    out = pl.pallas_call(
        _kernel,
        out_shape=jax.ShapeDtypeStruct((S, D), bf16),
        in_specs=[any_spec, any_spec, any_spec, any_spec, vmem_spec, any_spec, vmem_spec],
        out_specs=any_spec,
        scratch_shapes=[
            pltpu.VMEM((S, D), bf16),
            pltpu.VMEM((3, D, D), bf16),
            pltpu.VMEM((D, D), bf16),
            pltpu.VMEM((D, F), bf16),
            pltpu.VMEM((F, D), bf16),
            pltpu.VMEM((S, D), bf16),
            pltpu.VMEM((D // 128, S // 2, 128), u32),
            pltpu.VMEM((S // 128, D // 2, 128), u32),
            pltpu.VMEM((S // 128, D // 2, 128), u32),
            pltpu.VMEM((S // 128, D // 2, 128), u32),
            pltpu.VMEM((S, D), bf16),
        ] + [pltpu.VMEM((NT, 64, 128), u32) for _ in range(NU)]
          + [pltpu.VMEM((S, BQ), f32) for _ in range(NU)]
          + [
            pltpu.VMEM((NU, 1, BQ), f32),
            pltpu.SemaphoreType.DMA((S // RB1,)),
            pltpu.SemaphoreType.DMA((6,)),
            pltpu.SemaphoreType.DMA((S // RB3,)),
        ],
        compiler_params=pltpu.CompilerParams(vmem_limit_bytes=120 * 2**20),
        name="fused_block",
    )(A_x.reshape(S, D), A_wqkv, A_wo, B_w1, B_b1, B_w2, B_b2)
    return out.reshape(1, S, D)
```

```python
import math

import jax
import jax.numpy as jnp
from jax import lax
import jax.experimental.pallas as pl
import jax.experimental.pallas.tpu as pltpu

S, D, H, DH, F = 2048, 1024, 32, 32, 3584
DQ, FQ = D // 4, F // 4
BQ = 512
NU = S // BQ
CK = 128
NC = S // CK
NT = BQ // 128
RB1 = 256
R = 64
RB3 = 4 * R
NB = S // RB3
NJ = FQ // 128
NS = R // 16
EPS = 1e-5
QSCALE = (DH ** -0.5) * math.log2(math.e)

bf16, f32, u32 = jnp.bfloat16, jnp.float32, jnp.uint32

A_TERMS = (((0, 1), (3, 1)), ((2, 1), (3, 1)), ((0, 1),), ((3, 1),),
           ((0, 1), (1, 1)), ((2, 1), (0, -1)), ((1, 1), (3, -1)))
B_TERMS = (((0, 1), (3, 1)), ((0, 1),), ((1, 1), (3, -1)), ((2, 1), (0, -1)),
           ((3, 1),), ((0, 1), (1, 1)), ((2, 1), (3, 1)))
USES = (((0, 1), (3, 1)), ((2, 1), (3, -1)), ((1, 1), (3, 1)), ((0, 1), (2, 1)),
        ((0, -1), (1, 1)), ((3, 1),), ((0, 1),))
ORDER = (0, 5, 6, 1, 3, 2, 4)
N_USES = (4, 2, 2, 4)


def _layernorm(x):
    m = jnp.mean(x, axis=-1, keepdims=True)
    xc = x - m
    v = jnp.mean(xc * xc, axis=-1, keepdims=True)
    return xc * lax.rsqrt(v + EPS)


def _gelu2(x):
    c = math.sqrt(2.0 / math.pi)
    inner = x * (c + (c * 0.044715) * (x * x))
    return x + x * jnp.tanh(inner)


def _dot(a, b):
    return jnp.dot(a, b, preferred_element_type=f32)


def _lin(terms, get):
    v = None
    for q, sg in terms:
        x = get(q)
        v = x if v is None else (v + x if sg > 0 else v - x)
    return v


def _operands(terms, t, load, scale=None):
    q = [_lin(terms[t], lambda quad: load(2 * (quad // 2) + i, 2 * (quad % 2) + k))
         for i in range(2) for k in range(2)]
    if scale is not None:
        q = [x * scale for x in q]
    return [_lin(terms[s], lambda quad: q[quad]) for s in range(7)]


def _strassen2(product, init, done, acc, z):
    cnt = [0] * 4
    for t in ORDER:
        c = [None] * 4
        ci = [0] * 4
        for s in ORDER:
            m = product(t, s)
            for qi, sgi in USES[s]:
                c[qi] = m if c[qi] is None else (c[qi] + m if sgi > 0 else c[qi] - m)
                ci[qi] += 1
                if ci[qi] == N_USES[qi]:
                    i, k = divmod(qi, 2)
                    for q, sg in USES[t]:
                        a, b = 2 * (q // 2) + i, 2 * (q % 2) + k
                        if cnt[q] == 0:
                            w = c[qi] + init(a, b)
                        else:
                            old = acc[q][z + qi]
                            w = old + c[qi] if sg > 0 else old - c[qi]
                        if cnt[q] == N_USES[q] - 1:
                            done(a, b, w)
                        else:
                            acc[q][qi] = w
            yield
        for q, _ in USES[t]:
            cnt[q] += 1


def _positions(tasks):
    tot = sum(w for w, _ in tasks)
    c, out = 0, []
    for w, f in tasks:
        c += w
        out.append((c / tot, w, f))
    return out


def _merge(*lists):
    return [(w, f) for _, w, f in sorted([e for l in lists for e in _positions(l)], key=lambda e: e[0])]


def _take(gen, n):
    for _ in range(n):
        yield next(gen)


def _quad(a, k):
    return 2 * (a // 2) + k // 2, 2 * (a % 2) + k % 2


def _ldw(ref, *idx):
    rs = idx[-1]
    return ref.bitcast(u32)[(*idx[:-1], slice(rs.start // 2, rs.stop // 2), slice(None))]


def _as_bf16(w):
    return pltpu.bitcast(w, bf16)


def _rows(start, n):
    return pl.ds(start if isinstance(start, int) else pl.multiple_of(start, n), n)


class _Sched:
    def __init__(self, z):
        self.z = z
        self.pend = {}

    def gate(self, parts):
        for token in self.pend.values():
            tok = token()
            parts = [jnp.concatenate([jnp.where(self.z == 0, p[:8], tok), p[8:]], axis=0) for p in parts]
        self.pend = {}
        return parts

    def run(self, gen, side, n, lo=0.0, hi=1.0):
        side = _positions(side)
        k = i = 0
        for _ in gen:
            i += 1
            frac = (i / n - lo) / (hi - lo)
            while k < len(side) and side[k][0] <= frac + 1e-9:
                key, token = side[k][2]()
                self.pend[key] = token
                k += 1
        while k < len(side):
            key, token = side[k][2]()
            self.pend[key] = token
            k += 1


def _kernel(x_hbm, wqkv_hbm, wo_hbm, w1_hbm, b1_ref, w2_hbm, b2_ref, o_hbm,
            x_s, k_s, qt_s, vt_s, ot_s, ms_s, sem_x, sem_w, sem_o, *rest):
    rest = list(rest)
    take = lambda n: [rest.pop(0) for _ in range(n)]
    qms, sbs = take(NU), take(NU)
    woo, w1o, w2o = take(7), take(7), take(7)
    yo, go, oo = take(7), take(7), take(7)
    c_s = (take(4), take(4))
    g_s, y_s, on_s, acc = take(4), take(4), take(4), take(4)
    h_s, wo_s, w1_s, wb_s = take(4)
    n1 = S // RB1

    def prep_q(h, u):
        g = h // 4
        row = lax.broadcasted_iota(jnp.int32, (64, 128), 0) // (DH // 2)
        keep = row == (h % 4)
        for t in range(NT):
            q = qt_s.bitcast(u32)[u * NT + t, pl.ds(pl.multiple_of(g * 64, 64), 64), :]
            qms[u][t] = jnp.where(keep, q, jnp.zeros_like(q))

    def qk_chunk(h, u, c, m8, sched=None):
        kk = _ldw(k_s, h // 4, slice(c * CK, (c + 1) * CK))
        if sched is not None:
            (kk,) = sched.gate([kk])
        qm = jnp.concatenate([_as_bf16(qms[u][t]) for t in range(NT)], axis=1)
        s = _dot(_as_bf16(kk), qm)
        sbs[u][c * CK:(c + 1) * CK, :] = s
        for r in range(CK // 8):
            sr = s[r * 8:(r + 1) * 8]
            m8 = sr if m8 is None else jnp.maximum(m8, sr)
        return m8

    def pv_chunk(h, c, s, m, l8, acc):
        p = jnp.exp2(s - m)
        for r in reversed(range(CK // 8)):
            pr = p[r * 8:(r + 1) * 8]
            l8 = pr if l8 is None else l8 + pr
        vt = _ldw(vt_s, c // 2, h, slice((c % 2) * DH, (c % 2 + 1) * DH))
        o = _dot(_as_bf16(vt), p.astype(bf16))
        return l8, (o if acc is None else acc + o)

    def finish(h, u, l8, acc):
        l = jnp.sum(l8, axis=0, keepdims=True)
        res = (acc * (1.0 / l)).astype(bf16)
        for t in range(NT):
            ot_s[u * NT + t, pl.ds(pl.multiple_of(h * DH, DH), DH), :] = res[:, t * 128:(t + 1) * 128]

    def last_pv(u):
        m = ms_s[u, 0:1, :]
        l8 = acc = None
        for c in range(NC):
            l8, acc = pv_chunk(H - 1, c, sbs[u][c * CK:(c + 1) * CK, :], m, l8, acc)
            yield
        finish(H - 1, u, l8, acc)

    def xn_tile(ct, row, n):
        return ot_s.at[2 * ct + row // D, pl.ds(pl.multiple_of(row % D, n), n), :]

    def phase1(later):
        def x_copy(r):
            return pltpu.make_async_copy(
                x_hbm.at[pl.ds(r * RB1, RB1)], x_s.at[pl.ds(r * RB1, RB1)], sem_x.at[r])

        def wqkv_copy(j):
            return pltpu.make_async_copy(
                wqkv_hbm.at[:, pl.ds(j * D, D)], wb_s.at[pl.ds(j * D, D)], sem_w.at[j])

        x_copy(0).start()
        wqkv_copy(1).start()
        x_copy(0).wait()
        for r in range(1, n1):
            x_copy(r).start()
        wqkv_copy(1).wait()
        wqkv_copy(0).start()
        wqkv_copy(2).start()

        def p1a(r, carry):
            @pl.when(r > 0)
            def _():
                x_copy(r).wait()
            sub = 128
            for a in range(RB1 // sub):
                row = pl.multiple_of(r * RB1 + a * sub, sub)
                xn = _layernorm(x_s[pl.ds(row, sub), :].astype(f32)).astype(bf16)
                kk = _dot(xn, wb_s[D:2 * D, :]).astype(bf16)
                for g in range(D // 128):
                    xn_tile(g, row, sub)[...] = xn[:, g * 128:(g + 1) * 128]
                    k_s[g, pl.ds(row, sub), :] = kk[:, g * 128:(g + 1) * 128]
            return carry

        lax.fori_loop(0, n1, p1a, 0)

        wqkv_copy(0).wait()
        wqkv_copy(2).wait()
        for cp in later:
            cp.start()

        def p1b(r, carry):
            xn = jnp.concatenate([xn_tile(g, r * RB1, RB1)[...] for g in range(D // 128)], axis=1)
            q = _dot(xn, wb_s[0:D, :]) * QSCALE
            for t in range(RB1 // 128):
                qt_s[r * (RB1 // 128) + t] = q[t * 128:(t + 1) * 128, :].T.astype(bf16)
            v = _dot(xn, wb_s[2 * D:3 * D, :])
            for t in range(RB1 // 128):
                vt = v[t * 128:(t + 1) * 128, :].T.astype(bf16)
                vt_s[r, :, t * DH:(t + 1) * DH, :] = vt.reshape(H, DH, 128)
            return carry

        lax.fori_loop(0, n1, p1b, 0)

    def phase2(early):
        late = [w2_copy(0, D, 5), w2_copy(2 * D, D, 6)]
        for cp in late:
            cp.start()
        for u in range(NU):
            prep_q(0, u)
            m8 = None
            for c in range(NC):
                m8 = qk_chunk(0, u, c, m8)
            ms_s[u] = jnp.broadcast_to(jnp.max(m8, axis=0, keepdims=True), (8, BQ))
            prep_q(1, u)
        for cp in early + late:
            cp.wait()

        def w_task(ld, dst, row, col, t, scale=None):
            def f():
                for s, op in enumerate(_operands(B_TERMS, t, ld, scale)):
                    dst[t][s, col, _rows(row, 16), :] = op.astype(bf16)
                return id(dst[t]), lambda: dst[t].bitcast(u32)[0, col, _rows(row >> 1, 8), :]
            return 2 + len(B_TERMS[t]), f

        def tiled(src, ntile, row, col):
            return lambda a, k: _as_bf16(
                src.bitcast(u32)[k * ntile + col, _rows((a * DQ + row) >> 1, 8), :]).astype(f32)

        def w2_piece(row, n):
            return lambda a, k: wb_s[_rows(a * FQ + row, 16),
                                     k * DQ + n * 128:k * DQ + (n + 1) * 128].astype(f32)

        def attn_steps(h, sched):
            for u in range(NU):
                m = ms_s[u, 0:1, :]
                m8 = l8 = acc = None
                for c in range(NC):
                    s_old = sbs[u][c * CK:(c + 1) * CK, :]
                    m8 = qk_chunk(h + 1, u, c, m8, sched)
                    l8, acc = pv_chunk(h, c, s_old, m, l8, acc)
                    if c < NC - 1:
                        yield
                ms_s[u] = jnp.broadcast_to(jnp.max(m8, axis=0, keepdims=True), (8, BQ))
                prep_q(jnp.minimum(h + 2, H - 1), u)
                finish(h, u, l8, acc)

        def attn(h, carry):
            sched = _Sched(h >> 12)
            piece = jnp.minimum(h, 27)
            side = []
            row = jnp.minimum(h, 15) * 16
            side += [w_task(tiled(w1_s, NJ, row, j), w1o, row, j, t) for j in range(NJ) for t in range(7)]
            for a in range(2):
                row = piece * 32 + a * 16
                side += [w_task(w2_piece(row, n), w2o, row, n, t, 0.5) for n in range(2) for t in range(7)]
            row = jnp.minimum(h, 15) * 16
            side += [w_task(tiled(wo_s, 2, row, n), woo, row, n, t) for n in range(2) for t in range(7)]
            sched.run(attn_steps(h, sched), side, NU * (NC - 1))
            return carry

        lax.fori_loop(0, H - 1, attn, 0)

    def w2_copy(row, n, sem):
        return pltpu.make_async_copy(w2_hbm.at[pl.ds(row, n)], wb_s.at[pl.ds(row, n)], sem_w.at[sem])

    def tile_copies(src, dst, sem):
        return [pltpu.make_async_copy(src.at[:, pl.ds(c * 128, 128)], dst.at[c], sem_w.at[sem])
                for c in range(dst.shape[0])]

    copies = (tile_copies(wo_hbm, wo_s, 3) + tile_copies(w1_hbm, w1_s, 4)
              + [w2_copy(D, D, 7), w2_copy(3 * D, F - 3 * D, 8)])
    phase1(copies)
    phase2(copies)

    def back():
        def lhs(sched, ref, s, nk):
            parts = sched.gate([_ldw(ref, sched.z + s, kt, slice(0, R)) for kt in range(nk)])
            return jnp.concatenate([_as_bf16(p) for p in parts], axis=1)

        def rhs(ref, s, n, rows):
            return _as_bf16(_ldw(ref, s, n, slice(0, rows)))

        def op_task(dst, t, col, sl, ld, z):
            def f():
                for s, op in enumerate(_operands(A_TERMS, t, ld)):
                    dst[t][s, col, sl * 16:(sl + 1) * 16, :] = op.astype(bf16)
                return id(dst[t]), lambda: _ldw(dst[t], z, col, slice(sl * 16, sl * 16 + 16))
            return f

        def f32_token(ref, i, z, row=0):
            return id(ref), lambda: pltpu.bitcast(ref[z + i, row:row + 8, :], u32)

        def o_tasks(i, z):
            def tr(ct):
                def f():
                    for t in range(RB3 // 128):
                        tile = _as_bf16(_ldw(ot_s, i * (RB3 // 128) + t, slice(ct * 128, (ct + 1) * 128))).T
                        on_s[ct // 2][ct % 2, t * 128:(t + 1) * 128, :] = tile
                    return id(on_s[ct // 2]), lambda: _ldw(on_s[ct // 2], z + ct % 2, slice(0, 16))
                return f

            def ld(sl, kt):
                return lambda a, k: _as_bf16(
                    _ldw(on_s[k], z + kt, slice(a * R + sl * 16, a * R + sl * 16 + 16))).astype(f32)
            return [(30, tr(ct)) for ct in range(8)] + [
                (40, op_task(oo, t, kt, sl, ld(sl, kt), z))
                for sl in range(NS) for kt in range(2) for t in range(7)]

        def wo_gen(i, blk, sched):
            for n in range(2):
                cols = lambda k: slice(k * DQ + n * 128, k * DQ + (n + 1) * 128)

                def init(a, k):
                    return x_s[pl.ds(pl.multiple_of(blk * RB3 + a * R, R), R), cols(k)].astype(f32)

                def done(a, k, v):
                    h_s[i % 2, a * R:(a + 1) * R, cols(k)] = v

                yield from _strassen2(lambda t, s: _dot(lhs(sched, oo[t], s, 2), rhs(woo[t], s, n, DQ)),
                                      init, done, acc, sched.z)

        def y_tasks(i, z):
            def ln(a, sl):
                def f():
                    y = _layernorm(h_s[i % 2, a * R + sl * 16:a * R + (sl + 1) * 16, :])
                    for ct in range(8):
                        y_s[a][ct, sl * 16:(sl + 1) * 16, :] = y[:, ct * 128:(ct + 1) * 128]
                    return f32_token(y_s[a], 0, z, sl * 16)
                return f

            def ld(sl, kt):
                return lambda a, k: y_s[a][z + 2 * k + kt, sl * 16:(sl + 1) * 16, :]
            return ([(100, ln(a, sl)) for sl in range(NS) for a in range(4)],
                    [(25, op_task(yo, t, kt, sl, ld(sl, kt), z))
                     for sl in range(NS) for kt in range(2) for t in range(7)])

        def act_tasks(j, z):
            def act(a, k):
                def f():
                    q, qi = _quad(a, k)
                    g_s[q][j * 4 + qi] = _gelu2(c_s[j % 2][q][z + qi])
                    return f32_token(g_s[q], j * 4 + qi, z)
                return f
            return [(60, act(a, k)) for a in (2, 3, 0, 1) for k in (0, 2, 1, 3)]

        def gop_tasks(t, z):
            def ld(j, sl):
                return lambda a, k: g_s[_quad(a, k)[0]][z + j * 4 + _quad(a, k)[1], sl * 16:(sl + 1) * 16, :]
            return [(25, op_task(go, t, j, sl, ld(j, sl), z)) for j in range(NJ) for sl in range(NS)]

        def mlp1_gen(j, sched):
            bs = [b1_ref[pl.ds(k * FQ + j * 128, 128)].astype(f32).reshape(1, 128) for k in range(4)]

            def done(a, k, v):
                q, qi = _quad(a, k)
                c_s[j % 2][q][qi] = v

            yield from _strassen2(lambda t, s: _dot(lhs(sched, yo[t], s, 2), rhs(w1o[t], s, j, DQ)),
                                  lambda a, k: bs[k], done, acc, sched.z)

        def mlp2_gen(i, sched):
            b2 = b2_ref[...].astype(f32).reshape(1, D)
            for n in range(2):
                cols = lambda k: slice(k * DQ + n * 128, k * DQ + (n + 1) * 128)

                def init(a, k):
                    return h_s[i % 2, a * R:(a + 1) * R, cols(k)] + b2[:, cols(k)]

                def done(a, k, v):
                    x_s[pl.ds(pl.multiple_of(i * RB3 + a * R, R), R), cols(k)] = v.astype(bf16)

                yield from _strassen2(lambda t, s: _dot(lhs(sched, go[t], s, NJ), rhs(w2o[t], s, n, FQ)),
                                      init, done, acc, sched.z)

        def mlp1(sched):
            prev = []
            for j in range(NJ):
                sched.run(mlp1_gen(j, sched), prev, 49, 0.04, 1.0)
                prev = act_tasks(j, sched.z)
            return prev

        def out_copy(i):
            return pltpu.make_async_copy(
                x_s.at[pl.ds(i * RB3, RB3)], o_hbm.at[pl.ds(i * RB3, RB3)], sem_o.at[i])

        for u in range(NU):
            for _ in last_pv(u):
                pass
        sched = _Sched(0)
        for _, f in o_tasks(0, 0):
            f()
        for _ in wo_gen(0, 0, sched):
            pass
        for l in y_tasks(0, 0):
            for _, f in l:
                f()
        for _, f in o_tasks(1, 0):
            f()

        def p3(i, carry):
            sched = _Sched(i >> 12)
            z = sched.z
            prev = mlp1(sched)
            gen = wo_gen(i + 1, jnp.minimum(i + 1, NB - 1), sched)
            sched.run(_take(gen, 49), prev, 49, 0.04, 1.0)
            sched.run(_take(gen, 49), gop_tasks(ORDER[0], z), 49, 0.0, 0.9)
            gen = mlp2_gen(i, sched)
            lns, yops = y_tasks(i + 1, z)
            for p in range(7):
                side = gop_tasks(ORDER[p + 1], z) if p < 6 else lns[:8]
                sched.run(_take(gen, 7), side, 7, 0.0, 0.86)
            sched.run(_take(gen, 49), _merge(lns[8:] + yops, o_tasks(jnp.minimum(i + 2, NB - 1), z)),
                      49, 0.0, 0.95)
            out_copy(i).start()
            return carry

        lax.fori_loop(0, NB, p3, 0)
        for i in range(NB):
            out_copy(i).wait()

    back()


@jax.jit
def pallas_sequential_preLN__softmax_full_mha__mixer_channel_mlp__prompt_kernel(
    A_x: jax.Array,
    A_wqkv: jax.Array,
    A_wo: jax.Array,
    B_x: jax.Array,
    B_w1: jax.Array,
    B_b1: jax.Array,
    B_w2: jax.Array,
    B_b2: jax.Array,
):
    del B_x
    any_spec = pl.BlockSpec(memory_space=pl.ANY)
    vmem_spec = pl.BlockSpec(memory_space=pltpu.VMEM)
    V = pltpu.VMEM
    out = pl.pallas_call(
        _kernel,
        out_shape=jax.ShapeDtypeStruct((S, D), bf16),
        in_specs=[any_spec, any_spec, any_spec, any_spec, vmem_spec, any_spec, vmem_spec],
        out_specs=any_spec,
        scratch_shapes=[
            V((S, D), bf16),
            V((D // 128, S, 128), bf16),
            V((S // 128, D, 128), bf16),
            V((NC // 2, H, 2 * DH, 128), bf16),
            V((S // 128, D, 128), bf16),
            V((NU, 8, BQ), f32),
            pltpu.SemaphoreType.DMA((S // RB1,)),
            pltpu.SemaphoreType.DMA((9,)),
            pltpu.SemaphoreType.DMA((NB,)),
        ] + [V((NT, 64, 128), u32)] * NU + [V((S, BQ), f32)] * NU
          + [V((7, 2, DQ, 128), bf16)] * 7 + [V((7, NJ, DQ, 128), bf16)] * 7
          + [V((7, 2, FQ, 128), bf16)] * 7
          + [V((7, 2, R, 128), bf16)] * 7 + [V((7, NJ, R, 128), bf16)] * 7 + [V((7, 2, R, 128), bf16)] * 7
          + [V((4, R, 128), f32)] * 8 + [V((4 * NJ, R, 128), f32)] * 4 + [V((8, R, 128), f32)] * 4
          + [V((2, RB3, 128), bf16)] * 4 + [V((4, R, 128), f32)] * 4 + [V((2, RB3, D), f32), V((D // 128, D, 128), bf16), V((F // 128, D, 128), bf16),
             V((F, D), bf16)],
        compiler_params=pltpu.CompilerParams(vmem_limit_bytes=125 * 2**20),
        name="fused_block",
    )(A_x.reshape(S, D), A_wqkv, A_wo, B_w1, B_b1, B_w2, B_b2)
    return out.reshape(1, S, D)
```

```python
import math

import jax
import jax.numpy as jnp
from jax import lax
import jax.experimental.pallas as pl
import jax.experimental.pallas.tpu as pltpu

S, D, H, DH, F = 2048, 1024, 32, 32, 3584
EPS = 1e-5
QSCALE = (DH ** -0.5) * math.log2(math.e)

BQ = 512
NU = S // BQ
NT = BQ // 128
CK = 128
NC = S // CK

R = 64
RB = 4 * R
NB = S // RB
NS = R // 16
DQ, FQ = D // 4, F // 4
NJ = FQ // 128

bf16, f32, u32 = jnp.bfloat16, jnp.float32, jnp.uint32

A_TERMS = (((0, 1), (3, 1)), ((2, 1), (3, 1)), ((0, 1),), ((3, 1),),
           ((0, 1), (1, 1)), ((2, 1), (0, -1)), ((1, 1), (3, -1)))
B_TERMS = (((0, 1), (3, 1)), ((0, 1),), ((1, 1), (3, -1)), ((2, 1), (0, -1)),
           ((3, 1),), ((0, 1), (1, 1)), ((2, 1), (3, 1)))
USES = (((0, 1), (3, 1)), ((2, 1), (3, -1)), ((1, 1), (3, 1)), ((0, 1), (2, 1)),
        ((0, -1), (1, 1)), ((3, 1),), ((0, 1),))
N_USES = (4, 2, 2, 4)
ORDER = (0, 5, 6, 1, 3, 2, 4)


def _layernorm(x):
    m = jnp.mean(x, axis=-1, keepdims=True)
    xc = x - m
    v = jnp.mean(xc * xc, axis=-1, keepdims=True)
    return xc * lax.rsqrt(v + EPS)


def _gelu2(x):
    c = math.sqrt(2.0 / math.pi)
    inner = x * (c + (c * 0.044715) * (x * x))
    return x + x * jnp.tanh(inner)


def _dot(a, b):
    return jnp.dot(a, b, preferred_element_type=f32)


def _lin(terms, get):
    v = None
    for q, sign in terms:
        x = get(q)
        v = x if v is None else (v + x if sign > 0 else v - x)
    return v


def _operands(terms, t, load, scale=None):
    q = [_lin(terms[t], lambda quad: load(2 * (quad // 2) + i, 2 * (quad % 2) + k))
         for i in range(2) for k in range(2)]
    if scale is not None:
        q = [x * scale for x in q]
    return [_lin(terms[s], lambda quad: q[quad]) for s in range(7)]


def _strassen2(product, init, done, acc, z):
    cnt = [0] * 4
    for t in ORDER:
        c = [None] * 4
        ci = [0] * 4
        for s in ORDER:
            m = product(t, s)
            for qi, inner_sign in USES[s]:
                c[qi] = m if c[qi] is None else (c[qi] + m if inner_sign > 0 else c[qi] - m)
                ci[qi] += 1
                if ci[qi] == N_USES[qi]:
                    i, k = divmod(qi, 2)
                    for q, sign in USES[t]:
                        a, b = 2 * (q // 2) + i, 2 * (q % 2) + k
                        if cnt[q] == 0:
                            first = init(a, b)
                            w = c[qi] if first is None else c[qi] + first
                        else:
                            old = acc[q][z + qi]
                            w = old + c[qi] if sign > 0 else old - c[qi]
                        if cnt[q] == N_USES[q] - 1:
                            done(a, b, w)
                        else:
                            acc[q][qi] = w
            yield
        for q, _ in USES[t]:
            cnt[q] += 1


def _quad(a, k):
    return 2 * (a // 2) + k // 2, 2 * (a % 2) + k % 2


def _rows(start, n):
    return pl.ds(start if isinstance(start, int) else pl.multiple_of(start, n), n)


def _words(ref, *idx):
    rs = idx[-1]
    return ref.bitcast(u32)[(*idx[:-1], slice(rs.start // 2, rs.stop // 2), slice(None))]


def _as_bf16(words):
    return pltpu.bitcast(words, bf16)


def _join(parts):
    return jnp.concatenate([_as_bf16(p) for p in parts], axis=1)


def _positions(tasks):
    total = sum(w for w, _ in tasks)
    c, out = 0, []
    for w, f in tasks:
        c += w
        out.append((c / total, w, f))
    return out


def _merge(*lists):
    entries = sorted([e for tasks in lists for e in _positions(tasks)], key=lambda e: e[0])
    return [(w, f) for _, w, f in entries]


def _take(gen, n):
    for _ in range(n):
        yield next(gen)


def _drain(gen):
    for _ in gen:
        pass


def _run(tasks):
    for _, f in tasks:
        f()


class _Sched:
    def __init__(self, z):
        self.z = z
        self.pending = {}

    def gate(self, parts):
        tok = None
        for token in self.pending.values():
            tok = token() if tok is None else jnp.where(self.z == 0, tok, token())
        self.pending = {}
        if tok is None:
            return parts
        return [jnp.concatenate([jnp.where(self.z == 0, p[:8], tok), p[8:]], axis=0) for p in parts]

    def run(self, gen, side, n, lo=0.0, hi=1.0, deadlines=True):
        side = _positions(side)
        k = i = 0
        for _ in gen:
            i += 1
            frac = (i / n - lo) / (hi - lo)
            while k < len(side) and side[k][0] <= frac + 1e-9:
                self._do(side[k][2], deadlines)
                k += 1
        while k < len(side):
            self._do(side[k][2], deadlines)
            k += 1

    def _do(self, task, deadlines):
        out = task()
        if deadlines and out is not None:
            self.pending[out[0]] = out[1]


def _kernel(x_hbm, wqkv_hbm, wo_hbm, w1_hbm, b1_ref, w2_hbm, b2_ref, o_hbm,
            x_s, k_s, qt_s, vt_s, ot_s, ms_s, sem_x, sem_w, sem_o, *rest):
    rest = list(rest)
    take = lambda n: [rest.pop(0) for _ in range(n)]
    qms, sbs = take(NU), take(NU)
    woo, w1o, w2o = take(7), take(7), take(7)
    yo, go, oo = take(7), take(7), take(7)
    c_s = (take(4), take(4))
    g_s, y_s, on_s, acc = take(4), take(4), take(4), take(4)
    h_s, wo_s, w1_s, wk_s, wb_s = take(5)

    def lhs(sched, ref, s, nk):
        return _join(sched.gate([_words(ref, sched.z + s, kt, slice(0, R)) for kt in range(nk)]))

    def rhs(ref, s, n, rows):
        return _as_bf16(_words(ref, s, n, slice(0, rows)))

    def op_task(terms, dst, t, col, row, ld, z, scale=None):
        def f():
            for s, op in enumerate(_operands(terms, t, ld, scale)):
                dst[t][s, col, _rows(row, 16), :] = op.astype(bf16)
            if isinstance(row, int):
                return id(dst[t]), lambda: dst[t].bitcast(u32)[z, col, _rows(row >> 1, 8), :]
            return id(dst[t]), lambda: dst[t].bitcast(u32)[0, 0, 0:8, :]
        return f

    def f32_token(ref, i, z, row=0):
        return id(ref), lambda: pltpu.bitcast(ref[z + i, row:row + 8, :], u32)

    def weight_piece(src, kb, nb, row, col):
        return lambda a, k: src[_rows(a * kb + row, 16),
                                k * nb + col * 128:k * nb + (col + 1) * 128].astype(f32)

    def prep_q(h, u):
        g = h // 4
        row = lax.broadcasted_iota(jnp.int32, (64, 128), 0) // (DH // 2)
        keep = row == (h % 4)
        for t in range(NT):
            q = qt_s.bitcast(u32)[u * NT + t, _rows(g * 64, 64), :]
            qms[u][t] = jnp.where(keep, q, jnp.zeros_like(q))

    def qk_chunk(h, u, c, m8, sched=None):
        kk = _words(k_s, h // 4, slice(c * CK, (c + 1) * CK))
        if sched is not None:
            (kk,) = sched.gate([kk])
        s = _dot(_as_bf16(kk), _join([qms[u][t] for t in range(NT)]))
        sbs[u][c * CK:(c + 1) * CK, :] = s
        for r in range(CK // 8):
            sr = s[r * 8:(r + 1) * 8]
            m8 = sr if m8 is None else jnp.maximum(m8, sr)
        return m8

    def store_max(u, m8):
        ms_s[u] = jnp.broadcast_to(jnp.max(m8, axis=0, keepdims=True), (8, BQ))

    def pv_chunk(h, c, s, m, l8, o):
        p = jnp.exp2(s - m)
        for r in reversed(range(CK // 8)):
            pr = p[r * 8:(r + 1) * 8]
            l8 = pr if l8 is None else l8 + pr
        vt = _words(vt_s, c // 2, h, slice((c % 2) * DH, (c % 2 + 1) * DH))
        part = _dot(_as_bf16(vt), p.astype(bf16))
        return l8, (part if o is None else o + part)

    def finish(h, u, l8, o):
        l = jnp.sum(l8, axis=0, keepdims=True)
        res = (o * (1.0 / l)).astype(bf16)
        for t in range(NT):
            ot_s[u * NT + t, _rows(h * DH, DH), :] = res[:, t * 128:(t + 1) * 128]

    def last_pv(u):
        m = ms_s[u, 0:1, :]
        l8 = o = None
        for c in range(NC):
            l8, o = pv_chunk(H - 1, c, sbs[u][c * CK:(c + 1) * CK, :], m, l8, o)
            yield
        finish(H - 1, u, l8, o)

    def phase1(later):
        def x_copy(r):
            return pltpu.make_async_copy(
                x_hbm.at[pl.ds(r * RB, RB)], x_s.at[pl.ds(r * RB, RB)], sem_x.at[r])

        wk_copies = [pltpu.make_async_copy(wqkv_hbm.at[:, pl.ds(D + c * 128, 128)], wk_s.at[c],
                                           sem_w.at[6 + c // 4]) for c in range(8)]
        wq_copy, wv_copy = [pltpu.make_async_copy(wqkv_hbm.at[:, pl.ds(j * D, D)],
                                                  wb_s.at[pl.ds(j * D, D)], sem_w.at[j])
                            for j in (0, 2)]

        def x_tasks(blk, z):
            def ln(a, sl):
                def f():
                    row = a * R + sl * 16
                    y = _layernorm(x_s[_rows(blk * RB + row, 16), :].astype(f32))
                    for ct in range(8):
                        yt = y[:, ct * 128:(ct + 1) * 128]
                        y_s[a][ct, sl * 16:(sl + 1) * 16, :] = yt
                        ot_s[2 * ct + (blk >> 2), _rows((blk & 3) * RB + row, 16), :] = yt.astype(bf16)
                    return f32_token(y_s[a], 0, z, sl * 16)
                return f

            def ld(sl, kt):
                return lambda a, k: y_s[a][z + 2 * k + kt, sl * 16:(sl + 1) * 16, :]
            return [(100, ln(a, sl)) for sl in range(NS) for a in range(4)] + [
                (25, op_task(A_TERMS, w1o, t, 2 * kt + (blk >> 2), (blk & 3) * R + sl * 16, ld(sl, kt), z))
                for sl in range(NS) for kt in range(2) for t in range(7)]

        def wqv_tasks(r):
            base = 2 * D * (r >> 2) + (r & 3) * 64
            return [(25, op_task(B_TERMS, w2o, t, n, r * 64 + sl * 16,
                                 weight_piece(wb_s, DQ, DQ, base + sl * 16, n), 0))
                    for sl in range(4) for n in range(2) for t in range(7)]

        def k_gen(r, first, sched):
            for a in range(4):
                rows = _rows((r & 3) * (RB // 2) + a * (R // 2), R // 2)
                for n in range(first, first + 4):
                    parts = sched.gate([ot_s.bitcast(u32)[2 * ct + (r >> 2), rows, :] for ct in range(8)])
                    kk = _dot(_join(parts), _as_bf16(_words(wk_s, n, slice(0, D))))
                    k_s[n, _rows(r * RB + a * R, R), :] = kk.astype(bf16)
                    yield

        x_copy(0).start()
        for cp in wk_copies[:4]:
            cp.start()
        x_copy(1).start()
        for k in range(4):
            on_s[k][1] = jnp.zeros((RB, 128), bf16)
        x_copy(0).wait()
        _run(x_tasks(0, 0))
        for cp in wk_copies[:4]:
            cp.wait()
        x_copy(2).start()

        def k_low(r, carry):
            @pl.when(r < NB - 1)
            def _():
                x_copy(r + 1).wait()

            @pl.when(r < NB - 3)
            def _():
                x_copy(r + 3).start()

            @pl.when(r == 2)
            def _():
                for cp in wk_copies[4:]:
                    cp.start()

            @pl.when(r == 4)
            def _():
                wq_copy.start()
            sched = _Sched(r >> 12)
            sched.run(k_gen(r, 0, sched), x_tasks(jnp.minimum(r + 1, NB - 1), sched.z), 16, 0.1, 0.94)
            return carry

        def k_high(r, carry):
            @pl.when(r == 4)
            def _():
                wv_copy.wait()
            sched = _Sched(r >> 12)
            sched.run(k_gen(r, 4, sched), wqv_tasks(r), 16, 0.0, 0.94)
            return carry

        lax.fori_loop(0, NB, k_low, 0)
        for cp in wk_copies[4:] + [wq_copy]:
            cp.wait()
        wv_copy.start()
        lax.fori_loop(0, NB, k_high, 0)
        for cp in later:
            cp.start()

        def qv_gen(r, m, n, sched):
            def product(t, s):
                parts = sched.gate([w1o[t].bitcast(u32)[s, 2 * kt + (r >> 2), _rows((r & 3) * (R // 2), R // 2), :]
                                    for kt in range(2)])
                return _dot(_join(parts), _as_bf16(_words(w2o[t], s, n, slice(m * DQ, (m + 1) * DQ))))

            def done(a, k, v):
                on_s[k][n, a * R:(a + 1) * R, :] = (v * QSCALE if m == 0 else v).astype(bf16)

            yield from _strassen2(product, lambda a, k: None, done, acc, sched.z)

        def transpose_tasks(r, m, n, z):
            def tr(k):
                def f():
                    ct = 2 * k + n
                    for t in range(2):
                        tile = _as_bf16(_words(on_s[k], z + n, slice(t * 128, (t + 1) * 128))).T
                        if m == 0:
                            qt_s[2 * r + t, ct * 128:(ct + 1) * 128, :] = tile
                        else:
                            for e in range(4):
                                vt_s[r, 4 * ct + e, t * DH:(t + 1) * DH, :] = tile[e * DH:(e + 1) * DH]
                    if m == 0:
                        return id(qt_s), lambda: _words(qt_s, 2 * r, slice(ct * 128, ct * 128 + 16))
                    return id(vt_s), lambda: _words(vt_s, r, 4 * ct, slice(0, 16))
                return f
            return [(1, tr(k)) for k in (0, 2, 1, 3)]

        def qv(r, carry):
            sched = _Sched(r >> 12)
            prev = transpose_tasks(jnp.maximum(r - 1, 0), 1, 1, sched.z)
            for m in range(2):
                for n in range(2):
                    sched.run(qv_gen(r, m, n, sched), prev, 49, 0.05, 0.7)
                    prev = transpose_tasks(r, m, n, sched.z)
            return r

        last = lax.fori_loop(0, NB, qv, 0)
        _run(transpose_tasks(NB - 1, 1, 1, 0))
        return last

    def phase2(early):
        for u in range(NU):
            prep_q(0, u)
            m8 = None
            for c in range(NC):
                m8 = qk_chunk(0, u, c, m8)
            store_max(u, m8)
            prep_q(1, u)
        for cp in early:
            cp.wait()

        def w_task(ld, dst, row, col, t, scale=None):
            return 2 + len(B_TERMS[t]), op_task(B_TERMS, dst, t, col, row, ld, 0, scale)

        def steps(h, sched):
            for u in range(NU):
                m = ms_s[u, 0:1, :]
                m8 = l8 = o = None
                for c in range(NC):
                    s_old = sbs[u][c * CK:(c + 1) * CK, :]
                    m8 = qk_chunk(h + 1, u, c, m8, sched)
                    l8, o = pv_chunk(h, c, s_old, m, l8, o)
                    if c < NC - 1:
                        yield
                store_max(u, m8)
                prep_q(jnp.minimum(h + 2, H - 1), u)
                finish(h, u, l8, o)

        def head(h, carry):
            sched = _Sched(h >> 12)
            piece = jnp.minimum(h, FQ // 32 - 1)
            row = jnp.minimum(h, DQ // 16 - 1) * 16
            side = [w_task(weight_piece(w1_s, DQ, FQ, row, j), w1o, row, j, t)
                    for j in range(NJ) for t in range(7)]
            for a in range(2):
                row2 = piece * 32 + a * 16
                side += [w_task(weight_piece(wb_s, FQ, DQ, row2, n), w2o, row2, n, t, 0.5)
                         for n in range(2) for t in range(7)]
            side += [w_task(weight_piece(wo_s, DQ, DQ, row, n), woo, row, n, t)
                     for n in range(2) for t in range(7)]
            sched.run(steps(h, sched), side, NU * (NC - 1))
            return carry

        lax.fori_loop(0, H - 1, head, 0)

    def phase3(zero):
        def o_tasks(i, z, dst):
            def tr(ct):
                def f():
                    for t in range(RB // 128):
                        tile = _as_bf16(_words(ot_s, i * (RB // 128) + t, slice(ct * 128, (ct + 1) * 128))).T
                        on_s[ct // 2][ct % 2, t * 128:(t + 1) * 128, :] = tile
                    return id(on_s[ct // 2]), lambda: _words(on_s[ct // 2], z + ct % 2, slice(0, 16))
                return f

            def ld(sl, kt):
                return lambda a, k: _as_bf16(
                    _words(on_s[k], z + kt, slice(a * R + sl * 16, a * R + sl * 16 + 16))).astype(f32)
            return [(30, tr(ct)) for ct in range(8)] + [
                (40, op_task(A_TERMS, dst, t, kt, sl * 16, ld(sl, kt), z))
                for sl in range(NS) for kt in range(2) for t in range(7)]

        def wo_gen(i, blk, sched, src):
            for n in range(2):
                cols = lambda k: slice(k * DQ + n * 128, k * DQ + (n + 1) * 128)

                def init(a, k):
                    return x_s[_rows(blk * RB + a * R, R), cols(k)].astype(f32)

                def done(a, k, v):
                    h_s[i % 2, a * R:(a + 1) * R, cols(k)] = v

                yield from _strassen2(lambda t, s: _dot(lhs(sched, src[t], s, 2), rhs(woo[t], s, n, DQ)),
                                      init, done, acc, sched.z)

        def y_tasks(i, z):
            def ln(a, sl):
                def f():
                    y = _layernorm(h_s[i % 2, a * R + sl * 16:a * R + (sl + 1) * 16, :])
                    for ct in range(8):
                        y_s[a][ct, sl * 16:(sl + 1) * 16, :] = y[:, ct * 128:(ct + 1) * 128]
                    return f32_token(y_s[a], 0, z, sl * 16)
                return f

            def ld(sl, kt):
                return lambda a, k: y_s[a][z + 2 * k + kt, sl * 16:(sl + 1) * 16, :]
            return ([(100, ln(a, sl)) for sl in range(NS) for a in range(4)],
                    [(25, op_task(A_TERMS, yo, t, kt, sl * 16, ld(sl, kt), z))
                     for sl in range(NS) for kt in range(2) for t in range(7)])

        def act_tasks(j, z):
            def act(a, k):
                def f():
                    q, qi = _quad(a, k)
                    g_s[q][j * 4 + qi] = _gelu2(c_s[j % 2][q][z + qi])
                    return f32_token(g_s[q], j * 4 + qi, z)
                return f
            return [(60, act(a, k)) for a in (2, 3, 0, 1) for k in (0, 2, 1, 3)]

        def g_tasks(t, z):
            def ld(j, sl):
                return lambda a, k: g_s[_quad(a, k)[0]][z + j * 4 + _quad(a, k)[1], sl * 16:(sl + 1) * 16, :]
            return [(25, op_task(A_TERMS, go, t, j, sl * 16, ld(j, sl), z))
                    for j in range(NJ) for sl in range(NS)]

        def mlp1_gen(j, sched):
            bias = [b1_ref[pl.ds(k * FQ + j * 128, 128)].astype(f32).reshape(1, 128) for k in range(4)]

            def done(a, k, v):
                q, qi = _quad(a, k)
                c_s[j % 2][q][qi] = v

            yield from _strassen2(lambda t, s: _dot(lhs(sched, yo[t], s, 2), rhs(w1o[t], s, j, DQ)),
                                  lambda a, k: bias[k], done, acc, sched.z)

        def mlp2_gen(i, sched):
            b2 = b2_ref[...].astype(f32).reshape(1, D)
            for n in range(2):
                cols = lambda k: slice(k * DQ + n * 128, k * DQ + (n + 1) * 128)

                def init(a, k):
                    return h_s[i % 2, a * R:(a + 1) * R, cols(k)] + b2[:, cols(k)]

                def done(a, k, v):
                    x_s[_rows(i * RB + a * R, R), cols(k)] = v.astype(bf16)

                yield from _strassen2(lambda t, s: _dot(lhs(sched, go[t], s, NJ), rhs(w2o[t], s, n, FQ)),
                                      init, done, acc, sched.z)

        def out_copy(i):
            return pltpu.make_async_copy(
                x_s.at[pl.ds(i * RB, RB)], o_hbm.at[pl.ds(i * RB, RB)], sem_o.at[i])

        def as_tasks(gen, n):
            def step():
                next(gen)
            return [(1, step)] * n

        sched = _Sched(zero)
        pv = [last_pv(u) for u in range(NU)]
        _drain(pv[0])
        sched.run(pv[1], o_tasks(0, zero, go), NC, deadlines=False)
        gen = wo_gen(0, 0, sched, go)
        following = o_tasks(1, zero, oo)
        sched.run(_take(gen, 49), _merge(as_tasks(pv[2], NC), following[:24]), 49, 0.1, 1.0)
        _drain(pv[2])
        sched.run(_take(gen, 49), _merge(as_tasks(pv[3], NC), following[24:]), 49, 0.0, 0.9)
        _drain(pv[3])
        _drain(gen)
        lns, yops = y_tasks(0, zero)
        _run(lns + yops)

        def block(i, carry):
            sched = _Sched(i >> 12)
            z = sched.z
            prev = []
            for j in range(NJ):
                sched.run(mlp1_gen(j, sched), prev, 49, 0.06, 1.0)
                prev = act_tasks(j, z)
            gen = wo_gen(i + 1, jnp.minimum(i + 1, NB - 1), sched, oo)
            sched.run(_take(gen, 49), prev, 49, 0.06, 1.0)
            sched.run(_take(gen, 49), g_tasks(ORDER[0], z), 49, 0.0, 0.8)
            gen = mlp2_gen(i, sched)
            lns, yops = y_tasks(i + 1, z)
            for p in range(7):
                side = g_tasks(ORDER[p + 1], z) if p < 6 else lns[:6]
                sched.run(_take(gen, 7), side, 7, 0.0, 0.72)
            sched.run(_take(gen, 49), _merge(lns[6:] + yops, o_tasks(jnp.minimum(i + 2, NB - 1), z, oo)),
                      49, 0.0, 0.95)
            out_copy(i).start()
            return carry

        lax.fori_loop(0, NB, block, 0)
        for i in range(NB):
            out_copy(i).wait()

    copies = [pltpu.make_async_copy(wo_hbm, wo_s, sem_w.at[3]),
              pltpu.make_async_copy(w1_hbm, w1_s, sem_w.at[4]),
              pltpu.make_async_copy(w2_hbm, wb_s, sem_w.at[5])]
    last_block = phase1(copies)
    phase2(copies)
    phase3(last_block >> 12)


@jax.jit
def pallas_sequential_preLN__softmax_full_mha__mixer_channel_mlp__prompt_kernel(
    A_x: jax.Array,
    A_wqkv: jax.Array,
    A_wo: jax.Array,
    B_x: jax.Array,
    B_w1: jax.Array,
    B_b1: jax.Array,
    B_w2: jax.Array,
    B_b2: jax.Array,
):
    del B_x
    any_spec = pl.BlockSpec(memory_space=pl.ANY)
    vmem_spec = pl.BlockSpec(memory_space=pltpu.VMEM)
    V = pltpu.VMEM
    scratch = [
        V((S, D), bf16),
        V((D // 128, S, 128), bf16),
        V((S // 128, D, 128), bf16),
        V((NC // 2, H, 2 * DH, 128), bf16),
        V((S // 128, D, 128), bf16),
        V((NU, 8, BQ), f32),
        pltpu.SemaphoreType.DMA((NB,)),
        pltpu.SemaphoreType.DMA((8,)),
        pltpu.SemaphoreType.DMA((NB,)),
    ]
    scratch += [V((NT, 64, 128), u32)] * NU + [V((S, BQ), f32)] * NU
    scratch += [V((7, 2, DQ, 128), bf16)] * 7 + [V((7, NJ, DQ, 128), bf16)] * 7 + [V((7, 2, FQ, 128), bf16)] * 7
    scratch += [V((7, 2, R, 128), bf16)] * 7 + [V((7, NJ, R, 128), bf16)] * 7 + [V((7, 2, R, 128), bf16)] * 7
    scratch += [V((4, R, 128), f32)] * 8
    scratch += [V((4 * NJ, R, 128), f32)] * 4 + [V((8, R, 128), f32)] * 4
    scratch += [V((2, RB, 128), bf16)] * 4 + [V((4, R, 128), f32)] * 4
    scratch += [V((2, RB, D), f32), V((D, D), bf16), V((D, F), bf16), V((D // 128, D, 128), bf16),
                V((F, D), bf16)]
    out = pl.pallas_call(
        _kernel,
        out_shape=jax.ShapeDtypeStruct((S, D), bf16),
        in_specs=[any_spec, any_spec, any_spec, any_spec, vmem_spec, any_spec, vmem_spec],
        out_specs=any_spec,
        scratch_shapes=scratch,
        compiler_params=pltpu.CompilerParams(vmem_limit_bytes=125 * 2**20),
        name="fused_block",
    )(A_x.reshape(S, D), A_wqkv, A_wo, B_w1, B_b1, B_w2, B_b2)
    return out.reshape(1, S, D)
```
